```python
import os as _os
_os.environ.setdefault("JAX_PLATFORMS", "cpu")
import jax
import jax.numpy as jnp

def _softmax(x, axis=-1):
    return jax.nn.softmax(x, axis=axis)
def _gelu(x):
    return jax.nn.gelu(x, approximate=True)
def _silu(x):
    return jax.nn.silu(x)
def _sigmoid(x):
    return jax.nn.sigmoid(x)
def _layernorm(x, axis=-1, eps=1e-5):
    m = jnp.mean(x, axis=axis, keepdims=True)
    v = jnp.var(x, axis=axis, keepdims=True)
    return (x - m) / jnp.sqrt(v + eps)
def _scatter_add(tgt, idx, src, axis=0):
    return tgt.at[idx].add(src)
def _segment_sum(src, seg, n):
    return jax.ops.segment_sum(src, seg, n)
class _Rng:
    def __init__(self, key):
        self._k = key
    def _next(self):
        self._k, sub = jax.random.split(self._k)
        return sub
    def normal(self, shape):
        return jax.random.normal(self._next(), shape, dtype=jnp.bfloat16)
    def randint(self, lo, hi, shape):
        return jax.random.randint(self._next(), shape, lo, hi, dtype=jnp.int32)
    def uniform(self, shape, lo=0.0, hi=1.0):
        return jax.random.uniform(self._next(), shape, jnp.bfloat16, lo, hi)
    def permutation(self, n):
        return jax.random.permutation(self._next(), n)


kernel_name = 'standalone__linear_kernel_hedgehog__prompt'

def setup_inputs():
    _rng = _Rng(jax.random.key(int.from_bytes(__import__("os").urandom(4), "little")))
    _w = (lambda a: (lambda t: t.astype(jnp.bfloat16) if jnp.issubdtype(t.dtype, jnp.floating) else t)(jnp.asarray(a)))
    B, S, D, H = 1, 2048, 1024, 32
    Dh = D // H
    return {
        "x": _w((lambda *s: _rng.normal(s) * 0.4)(B, S, D)),
        "wqkv": _w((lambda *s: _rng.normal(s) * 0.4)(D, 3 * D)),
        "w_phi": _w((lambda *s: _rng.normal(s) * 0.4)(H, Dh, Dh) * (Dh ** -0.5)),
        "wo": _w((lambda *s: _rng.normal(s) * 0.05)(D, D)),
    }

def reference(x, wqkv, w_phi, wo):
    B, S, D = x.shape
    H = 32; Dh = D // H
    qkv = (lambda x, *d: x.transpose(*d))((x @ wqkv).reshape(B, S, 3, H, Dh), 2, 0, 3, 1, 4)
    q, k, v = qkv[0], qkv[1], qkv[2]
    pq = jnp.einsum("bhsd,hdf->bhsf", q, w_phi)
    pk = jnp.einsum("bhsd,hdf->bhsf", k, w_phi)
    phi_q = jnp.concatenate([_softmax(pq, axis=-1), _softmax(-pq, axis=-1)], axis=-1)
    phi_k = jnp.concatenate([_softmax(pk, axis=-1), _softmax(-pk, axis=-1)], axis=-1)
    kv = jnp.einsum("bhsf,bhsd->bhfd", phi_k, v)
    z  = jnp.einsum("bhsf->bhf", phi_k)
    num = jnp.einsum("bhqf,bhfd->bhqd", phi_q, kv)
    den = jnp.einsum("bhqf,bhf->bhq", phi_q, z)[..., None] + 1e-6
    o = num / den
    return (lambda x, *d: x.transpose(*d))(o, 0, 2, 1, 3).reshape(B, S, D) @ wo
```

```python
import contextlib
import math
import re

import jax
import jax.numpy as jnp
from jax import lax
from jax.experimental import pallas as pl
from jax.experimental.pallas import tpu as pltpu

S, D, H, DH = 2048, 1024, 32, 32
LOG2E = math.log2(math.e)
NT = (((1,), (1,)), ((), ()))
NN = (((1,), (0,)), ((), ()))
T = 512
NTILE = S // T
NSUB = T // 128
T2 = 512
ODMA = 4
OT = 'f32'
ZHEAD = 'sum'
ZLOOP = 'sum'
NP = H // 2
NG = 8
F32 = jnp.float32
BF16 = jnp.bfloat16
SCOPES = False

HEAD = "Wk0 FK0 FK1 Wk1 FK2 FK3 Wxa PKA0 Wk2 FK4 FK5 Wk3 FK6 FK7 PKB0 SM0 Wx0 PK1 SM1 PK2 Wv TV PK3 SM2 V0 V1 SM3 V2 V3 KVA ZU"
ORDER1 = "PK0 PK1 PK2 PK3 SM0 SM1 SM2 SM3 V0 V1 V2 V3 KV0 KV1 KV2 KV3 ZU"
MID = "Wq Wo FQ KVZ"
ORDER2 = "PQ0 PQ1 SM0 PQ2 SM1 PQ3 SM2 SM3 NUM0 NUM1 NUM2 NUM3 OUT0 OUT1 OUT2 OUT3"


def _scope(name):
    return jax.named_scope(name) if SCOPES else contextlib.nullcontext()


def _rcp(x):
    r = pl.reciprocal(x, approx=True)
    return r * (2.0 - x * r)


def _allreduce(v, op):
    ax = v.ndim - 2
    v = op(v, pltpu.roll(v, 4, ax))
    v = op(v, pltpu.roll(v, 2, ax))
    return v


def _exps(p):
    p4 = p.reshape(NP, 8, 8, 128)
    mx = _allreduce(jnp.max(p4, axis=1), jnp.maximum)[:, None]
    mn = _allreduce(jnp.min(p4, axis=1), jnp.minimum)[:, None]
    ep = jnp.exp2(p4 - mx)
    en = jnp.exp2(mn - p4)
    rp = _rcp(_allreduce(jnp.sum(ep, axis=1), jnp.add))
    rn = _rcp(_allreduce(jnp.sum(en, axis=1), jnp.add))
    return ep, en, rp, rn


NK = 8
S_WPHI, S_K0, S_XA, S_X0, S_V, S_X1, S_Q, S_OUT = 0, 1, 5, 6, 7, 8, 9, 10
S_XR, S_O = S_X1, S_Q
NSEM = 11


U32 = jnp.uint32


def _pk(x):
    return pltpu.bitcast(x, U32)


def _upk(x):
    return pltpu.bitcast(x, BF16)


def _run(jobs, order):
    for j in order.split():
        m = re.match(r"([A-Za-z]+)(\d*)(?::(\d+)/(\d+))?$", j)
        name, n, c, nc = m.groups()
        args = []
        if n:
            args.append(int(n))
        if c is not None:
            args += [int(c), int(nc)]
        jobs[name](*args)


def _kernel(x_hbm, wqkv_hbm, wphi_hbm, wo_hbm, o_hbm,
            x_v, wphi_v, rq_v, rk_v, rv_v, ro_v,
            wqT_ref, wkT_ref, wvT_ref, pkp_ref, kvacc_ref, zacc_ref, kvz_ref, ob_ref,
            sem):
    def xrows(lo, hi, s):
        return pltpu.make_async_copy(x_hbm.at[pl.ds(lo, hi - lo), :], x_v.at[pl.ds(lo, hi - lo), :],
                                     sem.at[s])

    cp_wphi = pltpu.make_async_copy(wphi_hbm, wphi_v, sem.at[S_WPHI])
    cp_xa = xrows(0, 128, S_XA)
    cp_x0 = xrows(128, T, S_X0)
    cp_x1 = xrows(T, 2 * T, S_X1)
    cp_xr = xrows(2 * T, S, S_XR)
    cp_k = [pltpu.make_async_copy(wqkv_hbm.at[pl.ds(j * 256, 256), pl.ds(D, D)],
                                  rk_v.at[pl.ds(j * 256, 256), :], sem.at[S_K0 + j]) for j in range(NK // 2)]
    cp_v = pltpu.make_async_copy(wqkv_hbm.at[:, pl.ds(2 * D, D)], rv_v, sem.at[S_V])
    cp_q = pltpu.make_async_copy(wqkv_hbm.at[:, pl.ds(0, D)], rq_v, sem.at[S_Q])
    cp_o = [pltpu.make_async_copy(wo_hbm.at[:, pl.ds(g * 128, 128)], ro_v.at[g], sem.at[S_O])
            for g in range(NG)]
    cp_wphi.start()
    for c in cp_k[:NK // 4]:
        c.start()
    cp_xa.start()
    for c in cp_k[NK // 4:]:
        c.start()
    cp_x0.start()
    cp_v.start()
    cp_x1.start()
    cp_q.start()
    cp_xr.start()
    for c in cp_o:
        c.start()

    r = lax.broadcasted_iota(jnp.int32, (128, DH), 0)
    c = lax.broadcasted_iota(jnp.int32, (128, DH), 1)
    sel = jnp.where(((r // 2) % DH) == c, 1.0, 0.0).astype(BF16)
    r = lax.broadcasted_iota(jnp.int32, (128, 128), 0)
    c = lax.broadcasted_iota(jnp.int32, (128, 128), 1)
    mask = (c // DH) == ((r // 64) * 2 + (r % 2))
    with _scope("w_wphi"):
        cp_wphi.wait()
    w2 = wphi_v[...].reshape(H * DH, DH)
    lall = lax.dot_general(sel, w2, NT, preferred_element_type=F32)
    lgs = [jnp.where(mask, lall[:, g * 128:(g + 1) * 128], 0.0).astype(BF16) for g in range(NG)]

    def fold_rows(raw, dstT, j):
        for g in range(NG):
            dstT[g * 64:(g + 1) * 64, j * 128:(j + 1) * 128] = _pk(
                (lax.dot_general(lgs[g], raw[j * 128:(j + 1) * 128, g * 128:(g + 1) * 128], NT,
                                 preferred_element_type=F32) * LOG2E).astype(BF16))

    def wait(name, cp):
        with _scope("w_" + name):
            cp.wait()

    def p1_jobs(base, first_tile):
        pk, phi, vt = {}, {}, {}
        zs = [None, None, False]

        def xs(n):
            return x_v[pl.ds(pl.multiple_of(base + n * 128, 128), 128), :] if not isinstance(base, int) \
                else x_v[base + n * 128:base + (n + 1) * 128, :]

        def PK(n):
            pk[n] = lax.dot_general(_upk(wkT_ref[...]), xs(n), NT, preferred_element_type=F32)

        def PKA(n):
            pkp_ref[...] = lax.dot_general(_upk(wkT_ref[:, 0:512]), xs(n)[:, 0:512], NT, preferred_element_type=F32)

        def PKB(n):
            pk[n] = pkp_ref[...] + lax.dot_general(_upk(wkT_ref[:, 512:D]), xs(n)[:, 512:D], NT,
                                            preferred_element_type=F32)

        def SM(n):
            ep, en, rp, rn = _exps(pk[n])
            php = (ep * rp[:, None]).reshape(NP, 64, 128)
            phn = (en * rn[:, None]).reshape(NP, 64, 128)
            phi[n] = [jnp.concatenate([php[p], phn[p]], axis=0).astype(BF16) for p in range(NP)]
            if (ZHEAD if first_tile else ZLOOP) == 'sum':
                zs[0] = php if zs[0] is None else zs[0] + php
                zs[1] = phn if zs[1] is None else zs[1] + phn
            elif first_tile and n == 0:
                zacc_ref[:, 0:64, :] = php
                zacc_ref[:, 64:128, :] = phn
            else:
                zacc_ref[:, 0:64, :] += php
                zacc_ref[:, 64:128, :] += phn

        def ZU():
            if zs[0] is None:
                return
            if first_tile and not zs[2]:
                zacc_ref[:, 0:64, :] = zs[0]
                zacc_ref[:, 64:128, :] = zs[1]
            else:
                zacc_ref[:, 0:64, :] += zs[0]
                zacc_ref[:, 64:128, :] += zs[1]
            zs[0] = zs[1] = None
            zs[2] = True

        def V(n):
            v32 = lax.dot_general(_upk(wvT_ref[...]), xs(n), NT, preferred_element_type=F32)
            vt[n] = [v32[p * 64:(p + 1) * 64].astype(BF16) for p in range(NP)]

        def KV(n, c=0, nc=1):
            for p in range(c * NP // nc, (c + 1) * NP // nc):
                upd = lax.dot_general(vt[n][p], phi[n][p], NT, preferred_element_type=F32)
                if first_tile and n == 0:
                    kvacc_ref[p] = upd
                else:
                    kvacc_ref[p] += upd

        def KVA(c=0, nc=1):
            for p in range(c * NP // nc, (c + 1) * NP // nc):
                upd = None
                for n in sorted(vt):
                    d = lax.dot_general(vt[n][p], phi[n][p], NT, preferred_element_type=F32)
                    upd = d if upd is None else upd + d
                if first_tile:
                    kvacc_ref[p] = upd
                else:
                    kvacc_ref[p] += upd

        def KVB(n):
            for p in range(NP):
                upd = (lax.dot_general(vt[n - 1][p], phi[n - 1][p], NT, preferred_element_type=F32)
                       + lax.dot_general(vt[n][p], phi[n][p], NT, preferred_element_type=F32))
                if first_tile and n == 1:
                    kvacc_ref[p] = upd
                else:
                    kvacc_ref[p] += upd

        return dict(PK=PK, PKA=PKA, PKB=PKB, SM=SM, V=V, KV=KV, KVA=KVA, KVB=KVB, ZU=ZU)

    with _scope("head"):
        jobs = p1_jobs(0, True)
        jobs["Wk"] = lambda j: wait(f"k{j}", cp_k[j])
        jobs["FK"] = lambda j: fold_rows(rk_v, wkT_ref, j)
        jobs["Wxa"] = lambda: wait("xa", cp_xa)
        jobs["Wx"] = lambda i: wait("x0", cp_x0)
        jobs["Wv"] = lambda: wait("v", cp_v)

        def TV():
            for g in range(NG):
                wvT_ref[g * 64:(g + 1) * 64, :] = _pk(rv_v[:, g * 128:(g + 1) * 128].T)
        jobs["TV"] = TV
        _run(jobs, HEAD)

    def p1(i, carry):
        _run(p1_jobs(i * T, False), ORDER1)
        return carry

    with _scope("p1loop"):
        wait("x1", cp_x1)
        wait("xr", cp_xr)
        lax.fori_loop(1, NTILE, p1, 0)

    def KVZ():
        r = lax.broadcasted_iota(jnp.int32, (64, 128), 0)
        c = lax.broadcasted_iota(jnp.int32, (64, 128), 1)
        kmask = (r // DH) == (c % 2)
        kvz_ref[...] = jnp.where(kmask[None], kvacc_ref[...], 0.0).astype(BF16)
        zacc_ref[...] = jnp.broadcast_to(jnp.sum(zacc_ref[...], axis=2, keepdims=True), zacc_ref.shape)

    def FQ():
        for j in range(NK):
            fold_rows(rq_v, wqT_ref, j)

    def Wo():
        for g in range(NG):
            cp_o[g].wait()

    with _scope("mid"):
        _run(dict(Wq=lambda: wait("q", cp_q), Wo=Wo, FQ=FQ, KVZ=KVZ), MID)

    def out_copy(i, n, h):
        row = pl.ds(pl.multiple_of(i * T2 + n * 128, 128), 128)
        col = pl.ds(h * (D // ODMA), D // ODMA)
        return pltpu.make_async_copy(ob_ref.at[row, col], o_hbm.at[row, col], sem.at[S_OUT])

    def p2(i, carry):
        base = i * T2
        pq, phi, ot, rden, o_nat = {}, {}, {}, {}, {}
        even = (lax.broadcasted_iota(jnp.int32, (NP, 8, 128), 1) % 2) == 0

        def PQ(n):
            xt = x_v[pl.ds(pl.multiple_of(base + n * 128, 128), 128), :]
            pq[n] = lax.dot_general(_upk(wqT_ref[...]), xt, NT, preferred_element_type=F32)

        def SM(n):
            ep, en, rp, rn = _exps(pq[n])
            zp = zacc_ref[:, 0:64, :].reshape(NP, 8, 8, 128)
            zn = zacc_ref[:, 64:128, :].reshape(NP, 8, 8, 128)
            den = _allreduce(jnp.sum(ep * zp, axis=1) * rp + jnp.sum(en * zn, axis=1) * rn, jnp.add)
            rd = _rcp(den + 1e-6)
            rot = pltpu.roll(rd, 1, 1)
            rden[n] = (jnp.where(even, rd, rot), jnp.where(even, rot, rd))
            php = (ep * rp[:, None]).reshape(NP, 64, 128)
            phn = (en * rn[:, None]).reshape(NP, 64, 128)
            phi[n] = [jnp.concatenate([php[p], phn[p]], axis=0).astype(BF16) for p in range(NP)]

        def NUM(n, c=0, nc=1):
            ot.setdefault(n, {})
            for p in range(c * NP // nc, (c + 1) * NP // nc):
                nd = lax.dot_general(kvz_ref[p], phi[n][p], NN, preferred_element_type=F32)
                oa = nd[0:32].reshape(4, 8, 128) * rden[n][0][p][None]
                ob = nd[32:64].reshape(4, 8, 128) * rden[n][1][p][None]
                ot[n][p] = jnp.concatenate([oa.reshape(32, 128), ob.reshape(32, 128)], axis=0)

        def OUT(n, c=0, nc=1):
            if n not in o_nat:
                o32 = jnp.concatenate([ot[n][p] for p in range(NP)], axis=0)
                o_nat[n] = o32.astype(BF16).T if OT == 'bf16' else o32.T.astype(BF16)
            row = pl.ds(pl.multiple_of(base + n * 128, 128), 128)
            for g in range(c * NG // nc, (c + 1) * NG // nc):
                res = lax.dot_general(o_nat[n], ro_v[g], NN, preferred_element_type=F32)
                ob_ref[row, g * 128:(g + 1) * 128] = res.astype(BF16)
                if (g + 1) % (NG // ODMA) == 0:
                    out_copy(i, n, g // (NG // ODMA)).start()

        _run(dict(PQ=PQ, SM=SM, NUM=NUM, OUT=OUT), ORDER2)
        return carry

    with _scope("p2loop"):
        lax.fori_loop(0, S // T2, p2, 0)
    with _scope("tail"):
        for i in range(S // T2):
            for n in range(T2 // 128):
                for h in range(ODMA):
                    out_copy(i, n, h).wait()


@jax.jit
def pallas_standalone__linear_kernel_hedgehog__prompt_kernel(x, wqkv, w_phi, wo):
    b, s, d = x.shape
    x2 = x.reshape(s, d)
    any_spec = pl.BlockSpec(memory_space=pl.ANY)
    out = pl.pallas_call(
        _kernel,
        out_shape=jax.ShapeDtypeStruct((s, d), x.dtype),
        in_specs=[any_spec] * 4,
        out_specs=any_spec,
        scratch_shapes=[
            pltpu.VMEM((S, D), BF16),
            pltpu.VMEM((H, DH, DH), BF16),
            pltpu.VMEM((D, D), BF16),
            pltpu.VMEM((D, D), BF16),
            pltpu.VMEM((D, D), BF16),
            pltpu.VMEM((NG, D, 128), BF16),
            pltpu.VMEM((D // 2, D), U32),
            pltpu.VMEM((D // 2, D), U32),
            pltpu.VMEM((D // 2, D), U32),
            pltpu.VMEM((D, 128), F32),
            pltpu.VMEM((NP, 64, 128), F32),
            pltpu.VMEM((NP, 128, 128), F32),
            pltpu.VMEM((NP, 64, 128), BF16),
            pltpu.VMEM((S, D), BF16),
            pltpu.SemaphoreType.DMA((NSEM,)),
        ],
        compiler_params=pltpu.CompilerParams(vmem_limit_bytes=100 * 1024 * 1024),
    )(x2, wqkv, w_phi, wo)
    return out.reshape(b, s, d)
```

```python
import math

import jax
import jax.numpy as jnp
from jax import lax
from jax.experimental import pallas as pl
from jax.experimental.pallas import tpu as pltpu

S, D, H, DH = 2048, 1024, 32, 32
NP = H // 2
NG = D // 128
T = 512
NSUB = T // 128
ODMA = 8
LOG2E = math.log2(math.e)
F32 = jnp.float32
BF16 = jnp.bfloat16
U32 = jnp.uint32
NT = (((1,), (1,)), ((), ()))
NN = (((1,), (0,)), ((), ()))

S_WPHI, S_K0, S_XA, S_X0, S_V, S_X1, S_Q, S_OUT = 0, 1, 5, 6, 7, 8, 9, 10
NSEM = 11


def _dot(a, b, dn):
    return lax.dot_general(a, b, dn, preferred_element_type=F32)


def _rcp(x):
    r = pl.reciprocal(x, approx=True)
    return r * (2.0 - x * r)


def _allreduce(v, op):
    v = op(v, pltpu.roll(v, 4, 1))
    v = op(v, pltpu.roll(v, 2, 1))
    return v


def _exps(p, sums=False):
    p4 = p.reshape(NP, 8, 8, 128)
    mx = _allreduce(jnp.max(p4, axis=1), jnp.maximum)[:, None]
    mn = _allreduce(jnp.min(p4, axis=1), jnp.minimum)[:, None]
    ep = jnp.exp2(p4 - mx)
    en = jnp.exp2(mn - p4)
    sp = _allreduce(jnp.sum(ep, axis=1), jnp.add)
    sn = _allreduce(jnp.sum(en, axis=1), jnp.add)
    if sums:
        return ep, en, sp, sn
    return ep, en, _rcp(sp), _rcp(sn)


def _pack(x):
    return pltpu.bitcast(x, U32)


def _unpack(x):
    return pltpu.bitcast(x, BF16)


def _kernel(x_hbm, wqkv_hbm, wphi_hbm, wo_hbm, o_hbm,
            x_v, wphi_v, rq_v, rk_v, rv_v, ro_v,
            wqT_ref, wkT_ref, wvT_ref, pkp_ref, kvacc_ref, zacc_ref, kvz_ref, ob_ref,
            sem):
    def xrows(lo, hi, s):
        return pltpu.make_async_copy(
            x_hbm.at[pl.ds(lo, hi - lo), :], x_v.at[pl.ds(lo, hi - lo), :], sem.at[s])

    cp_wphi = pltpu.make_async_copy(wphi_hbm, wphi_v, sem.at[S_WPHI])
    cp_xa = xrows(0, 128, S_XA)
    cp_x0 = xrows(128, T, S_X0)
    cp_x1 = xrows(T, 2 * T, S_X1)
    cp_xr = xrows(2 * T, S, S_X1)
    cp_k = [pltpu.make_async_copy(wqkv_hbm.at[pl.ds(j * 256, 256), pl.ds(D, D)],
                                  rk_v.at[pl.ds(j * 256, 256), :], sem.at[S_K0 + j])
            for j in range(4)]
    cp_v = pltpu.make_async_copy(wqkv_hbm.at[:, pl.ds(2 * D, D)], rv_v, sem.at[S_V])
    cp_q = pltpu.make_async_copy(wqkv_hbm.at[:, pl.ds(0, D)], rq_v, sem.at[S_Q])
    cp_o = [pltpu.make_async_copy(wo_hbm.at[:, pl.ds(g * 128, 128)], ro_v.at[g], sem.at[S_Q])
            for g in range(NG)]
    for c in [cp_wphi, cp_k[0], cp_k[1], cp_xa, cp_k[2], cp_k[3], cp_x0, cp_v, cp_x1, cp_q,
              cp_xr] + cp_o:
        c.start()

    r = lax.broadcasted_iota(jnp.int32, (128, DH), 0)
    c = lax.broadcasted_iota(jnp.int32, (128, DH), 1)
    sel = jnp.where(((r // 2) % DH) == c, 1.0, 0.0).astype(BF16)
    r = lax.broadcasted_iota(jnp.int32, (128, 128), 0)
    c = lax.broadcasted_iota(jnp.int32, (128, 128), 1)
    mask = (c // DH) == ((r // 64) * 2 + (r % 2))
    cp_wphi.wait()
    w2 = wphi_v[...].reshape(H * DH, DH)
    lall = _dot(sel, w2, NT)
    lgs = [jnp.where(mask, lall[:, g * 128:(g + 1) * 128], 0.0).astype(BF16) for g in range(NG)]

    def fold_rows(raw, dstT, j):
        for g in range(NG):
            blk = raw[j * 128:(j + 1) * 128, g * 128:(g + 1) * 128]
            dstT[g * 64:(g + 1) * 64, j * 128:(j + 1) * 128] = _pack(
                (_dot(lgs[g], blk, NT) * LOG2E).astype(BF16))

    class KTile:
        def __init__(self, base, first):
            self.base, self.first = base, first
            self.pk, self.phi, self.vt = {}, {}, {}
            self.zp = self.zn = None

        def xs(self, n):
            lo = self.base + n * 128
            if isinstance(lo, int):
                return x_v[lo:lo + 128, :]
            return x_v[pl.ds(pl.multiple_of(lo, 128), 128), :]

        def proj_k(self, n):
            self.pk[n] = _dot(_unpack(wkT_ref[...]), self.xs(n), NT)

        def proj_k_lo(self, n):
            pkp_ref[...] = _dot(_unpack(wkT_ref[:, 0:512]), self.xs(n)[:, 0:512], NT)

        def proj_k_hi(self, n):
            self.pk[n] = pkp_ref[...] + _dot(_unpack(wkT_ref[:, 512:D]), self.xs(n)[:, 512:D], NT)

        def features(self, n):
            ep, en, rp, rn = _exps(self.pk[n])
            php = (ep * rp[:, None]).reshape(NP, 64, 128)
            phn = (en * rn[:, None]).reshape(NP, 64, 128)
            self.phi[n] = [jnp.concatenate([php[p], phn[p]], axis=0).astype(BF16)
                           for p in range(NP)]
            self.zp = php if self.zp is None else self.zp + php
            self.zn = phn if self.zn is None else self.zn + phn

        def proj_v(self, n):
            v32 = _dot(_unpack(wvT_ref[...]), self.xs(n), NT)
            self.vt[n] = [v32[p * 64:(p + 1) * 64].astype(BF16) for p in range(NP)]

        def kv_one(self, n):
            for p in range(NP):
                kvacc_ref[p] += _dot(self.vt[n][p], self.phi[n][p], NT)

        def kv_init(self):
            for p in range(NP):
                upd = None
                for n in range(NSUB):
                    d = _dot(self.vt[n][p], self.phi[n][p], NT)
                    upd = d if upd is None else upd + d
                kvacc_ref[p] = upd

        def z_update(self):
            if self.first:
                zacc_ref[:, 0:64, :] = self.zp
                zacc_ref[:, 64:128, :] = self.zn
            else:
                zacc_ref[:, 0:64, :] += self.zp
                zacc_ref[:, 64:128, :] += self.zn

    t0 = KTile(0, True)
    cp_k[0].wait()
    fold_rows(rk_v, wkT_ref, 0)
    fold_rows(rk_v, wkT_ref, 1)
    cp_k[1].wait()
    fold_rows(rk_v, wkT_ref, 2)
    fold_rows(rk_v, wkT_ref, 3)
    cp_xa.wait()
    t0.proj_k_lo(0)
    cp_k[2].wait()
    fold_rows(rk_v, wkT_ref, 4)
    fold_rows(rk_v, wkT_ref, 5)
    cp_k[3].wait()
    fold_rows(rk_v, wkT_ref, 6)
    fold_rows(rk_v, wkT_ref, 7)
    t0.proj_k_hi(0)
    t0.features(0)
    cp_x0.wait()
    t0.proj_k(1)
    t0.features(1)
    t0.proj_k(2)
    cp_v.wait()
    for g in range(NG):
        wvT_ref[g * 64:(g + 1) * 64, :] = _pack(rv_v[:, g * 128:(g + 1) * 128].T)
    t0.proj_k(3)
    t0.features(2)
    t0.proj_v(0)
    t0.proj_v(1)
    t0.features(3)
    t0.proj_v(2)
    t0.proj_v(3)
    t0.kv_init()
    t0.z_update()

    def k_step(i, carry):
        t = KTile(T + i * T, False)
        for n in range(NSUB):
            t.proj_k(n)
        for n in range(NSUB):
            t.features(n)
        for n in range(NSUB):
            t.proj_v(n)
        for n in range(NSUB):
            t.kv_one(n)
        t.z_update()
        return carry

    cp_x1.wait()
    cp_xr.wait()
    lax.fori_loop(0, S // T - 1, k_step, 0)

    cp_q.wait()
    for c in cp_o:
        c.wait()
    for j in range(NG):
        fold_rows(rq_v, wqT_ref, j)
    r = lax.broadcasted_iota(jnp.int32, (64, 128), 0)
    c = lax.broadcasted_iota(jnp.int32, (64, 128), 1)
    kmask = (r // DH) == (c % 2)
    kvz_ref[...] = jnp.where(kmask[None], kvacc_ref[...], 0.0).astype(BF16)
    zacc_ref[...] = jnp.broadcast_to(jnp.sum(zacc_ref[...], axis=2, keepdims=True),
                                     zacc_ref.shape)

    def out_copy(i, n, h):
        row = pl.ds(pl.multiple_of(i * T + n * 128, 128), 128)
        col = pl.ds(h * (D // ODMA), D // ODMA)
        return pltpu.make_async_copy(ob_ref.at[row, col], o_hbm.at[row, col], sem.at[S_OUT])

    def q_step(i, carry):
        base = i * T
        pq, phi, ot, rden = {}, {}, {}, {}
        even = (lax.broadcasted_iota(jnp.int32, (NP, 8, 128), 1) % 2) == 0

        def proj_q(n):
            xt = x_v[pl.ds(pl.multiple_of(base + n * 128, 128), 128), :]
            pq[n] = _dot(_unpack(wqT_ref[...]), xt, NT)

        def features(n):
            ep, en, sp, sn = _exps(pq[n], True)
            zp = zacc_ref[:, 0:64, :].reshape(NP, 8, 8, 128)
            zn = zacc_ref[:, 64:128, :].reshape(NP, 8, 8, 128)
            rp = _rcp(sp)
            en = en * (sp * _rcp(sn))[:, None]
            den = _allreduce(jnp.sum(ep * zp, axis=1) + jnp.sum(en * zn, axis=1), jnp.add)
            rd = rp * _rcp(rp * den + 1e-6)
            rot = pltpu.roll(rd, 1, 1)
            rden[n] = (jnp.where(even, rd, rot), jnp.where(even, rot, rd))
            php = ep.reshape(NP, 64, 128)
            phn = en.reshape(NP, 64, 128)
            phi[n] = [jnp.concatenate([php[p], phn[p]], axis=0).astype(BF16) for p in range(NP)]

        def attend(n):
            ot[n] = []
            for p in range(NP):
                nd = _dot(kvz_ref[p], phi[n][p], NN)
                oa = nd[0:32].reshape(4, 8, 128) * rden[n][0][p][None]
                ob = nd[32:64].reshape(4, 8, 128) * rden[n][1][p][None]
                ot[n].append(jnp.concatenate([oa.reshape(32, 128), ob.reshape(32, 128)], axis=0))

        def project(n):
            o_nat = jnp.concatenate(ot[n], axis=0).T.astype(BF16)
            row = pl.ds(pl.multiple_of(base + n * 128, 128), 128)
            for g in range(NG):
                ob_ref[row, g * 128:(g + 1) * 128] = _dot(o_nat, ro_v[g], NN).astype(BF16)
                if (g + 1) % (NG // ODMA) == 0:
                    out_copy(i, n, g // (NG // ODMA)).start()

        proj_q(0); proj_q(1); features(0)
        proj_q(2); attend(0); features(1)
        proj_q(3); attend(1); features(2)
        project(0); attend(2); features(3)
        project(1); attend(3); project(2); project(3)
        return carry

    lax.fori_loop(0, S // T, q_step, 0)
    for i in range(S // T):
        for n in range(NSUB):
            for h in range(ODMA):
                out_copy(i, n, h).wait()


@jax.jit
def pallas_standalone__linear_kernel_hedgehog__prompt_kernel(
    x: jax.Array,
    wqkv: jax.Array,
    w_phi: jax.Array,
    wo: jax.Array,
):
    b, s, d = x.shape
    assert (b, s, d) == (1, S, D) and w_phi.shape == (H, DH, DH)
    any_spec = pl.BlockSpec(memory_space=pl.ANY)
    out = pl.pallas_call(
        _kernel,
        out_shape=jax.ShapeDtypeStruct((s, d), x.dtype),
        in_specs=[any_spec] * 4,
        out_specs=any_spec,
        scratch_shapes=[
            pltpu.VMEM((S, D), BF16),
            pltpu.VMEM((H, DH, DH), BF16),
            pltpu.VMEM((D, D), BF16),
            pltpu.VMEM((D, D), BF16),
            pltpu.VMEM((D, D), BF16),
            pltpu.VMEM((NG, D, 128), BF16),
            pltpu.VMEM((D // 2, D), U32),
            pltpu.VMEM((D // 2, D), U32),
            pltpu.VMEM((D // 2, D), U32),
            pltpu.VMEM((D, 128), F32),
            pltpu.VMEM((NP, 64, 128), F32),
            pltpu.VMEM((NP, 128, 128), F32),
            pltpu.VMEM((NP, 64, 128), BF16),
            pltpu.VMEM((S, D), BF16),
            pltpu.SemaphoreType.DMA((NSEM,)),
        ],
        compiler_params=pltpu.CompilerParams(vmem_limit_bytes=100 * 1024 * 1024),
    )(x.reshape(s, d), wqkv, w_phi, wo)
    return out.reshape(b, s, d)
```
